```python
import os as _os
_os.environ.setdefault("JAX_PLATFORMS", "cpu")
import jax
import jax.numpy as jnp

def _softmax(x, axis=-1):
    return jax.nn.softmax(x, axis=axis)
def _gelu(x):
    return jax.nn.gelu(x, approximate=True)
def _silu(x):
    return jax.nn.silu(x)
def _sigmoid(x):
    return jax.nn.sigmoid(x)
def _layernorm(x, axis=-1, eps=1e-5):
    m = jnp.mean(x, axis=axis, keepdims=True)
    v = jnp.var(x, axis=axis, keepdims=True)
    return (x - m) / jnp.sqrt(v + eps)
def _scatter_add(tgt, idx, src, axis=0):
    return tgt.at[idx].add(src)
def _segment_sum(src, seg, n):
    return jax.ops.segment_sum(src, seg, n)
class _Rng:
    def __init__(self, key):
        self._k = key
    def _next(self):
        self._k, sub = jax.random.split(self._k)
        return sub
    def normal(self, shape):
        return jax.random.normal(self._next(), shape, dtype=jnp.bfloat16)
    def randint(self, lo, hi, shape):
        return jax.random.randint(self._next(), shape, lo, hi, dtype=jnp.int32)
    def uniform(self, shape, lo=0.0, hi=1.0):
        return jax.random.uniform(self._next(), shape, jnp.bfloat16, lo, hi)
    def permutation(self, n):
        return jax.random.permutation(self._next(), n)


kernel_name = 'standalone__mha_softmax__near_ridge'

def setup_inputs():
    _rng = _Rng(jax.random.key(int.from_bytes(__import__("os").urandom(4), "little")))
    _w = (lambda a: (lambda t: t.astype(jnp.bfloat16) if jnp.issubdtype(t.dtype, jnp.floating) else t)(jnp.asarray(a)))
    B, H, Sq, Sk, D = 16, 16, 256, 256, 256
    return {
        "q": _w((lambda *s: _rng.normal(s) * 0.4)(B, H, Sq, D)),
        "k": _w((lambda *s: _rng.normal(s) * 0.4)(B, H, Sk, D)),
        "v": _w((lambda *s: _rng.normal(s) * 0.05)(B, H, Sk, D)),
    }

def reference(q, k, v):
    scale = q.shape[-1] ** -0.5
    scores = jnp.einsum("bhqd,bhkd->bhqk", q, k) * scale
    p = _softmax(scores, axis=-1)
    return jnp.einsum("bhqk,bhkd->bhqd", p, v)
```

```python
import functools

import jax
import jax.numpy as jnp
import jax.experimental.pallas as pl
import jax.experimental.pallas.tpu as pltpu

_LOG2E = 1.4426950408889634
_C = 2
_R = 8
_BACK = 2


def _attention_head(q, k, v, scale):
    s = jax.lax.dot_general(
        q, k, (((1,), (1,)), ((), ())), preferred_element_type=jnp.float32)
    m = jnp.max(s, axis=-1, keepdims=True)
    p = jnp.exp2((s - m) * (scale * _LOG2E))
    l = jnp.sum(p, axis=-1, keepdims=True)
    o = jnp.dot(p.astype(v.dtype), v, preferred_element_type=jnp.float32)
    return o * (1.0 / l)


def _kernel(q_hbm, k_hbm, v_hbm, o_hbm, q_buf, k_buf, v_buf, o_buf, in_sem,
            out_sem, *, chunk, ring, n_chunks, bulk_at, scale):
    streams = ((q_hbm, q_buf), (k_hbm, k_buf), (v_hbm, v_buf))

    def loads(i, slot):
        return [
            pltpu.make_async_copy(
                src.at[pl.ds(i * chunk, chunk)], dst.at[slot],
                in_sem.at[a * ring + slot])
            for a, (src, dst) in enumerate(streams)
        ]

    def store(h0, n, j):
        return pltpu.make_async_copy(
            o_buf.at[pl.ds(h0, n)], o_hbm.at[pl.ds(h0, n)], out_sem.at[j])

    n_bulk = bulk_at * chunk
    bulk = store(0, n_bulk, 0)
    tail = store(n_bulk, n_chunks * chunk - n_bulk, 1)

    for i in range(ring):
        for cp in loads(i, i):
            cp.start()

    def step(i, carry):
        slot = i % ring
        for cp in loads(i, slot):
            cp.wait()

        @pl.when(i == bulk_at)
        def _():
            bulk.start()

        for h in range(chunk):
            o = _attention_head(q_buf[slot, h], k_buf[slot, h], v_buf[slot, h], scale)
            o_buf[i * chunk + h] = o.astype(o_buf.dtype)

        @pl.when(i + ring < n_chunks)
        def _():
            for cp in loads(i + ring, slot):
                cp.start()

        return carry

    jax.lax.fori_loop(0, n_chunks, step, 0)
    tail.start()
    bulk.wait()
    tail.wait()


@jax.jit
def pallas_standalone__mha_softmax__near_ridge_kernel(
    q: jax.Array,
    k: jax.Array,
    v: jax.Array,
):
    b, h, sq, d = q.shape
    sk = k.shape[2]
    n_heads = b * h
    n_chunks = n_heads // _C
    assert n_chunks * _C == n_heads and n_chunks > _R > _BACK >= 1

    any_spec = pl.BlockSpec(memory_space=pl.ANY)
    out = pl.pallas_call(
        functools.partial(
            _kernel, chunk=_C, ring=_R, n_chunks=n_chunks,
            bulk_at=n_chunks - _BACK, scale=d ** -0.5),
        in_specs=[any_spec, any_spec, any_spec],
        out_specs=any_spec,
        out_shape=jax.ShapeDtypeStruct((n_heads, sq, d), q.dtype),
        scratch_shapes=[
            pltpu.VMEM((_R, _C, sq, d), q.dtype),
            pltpu.VMEM((_R, _C, sk, d), k.dtype),
            pltpu.VMEM((_R, _C, sk, d), v.dtype),
            pltpu.VMEM((n_heads, sq, d), q.dtype),
            pltpu.SemaphoreType.DMA((3 * _R,)),
            pltpu.SemaphoreType.DMA((2,)),
        ],
        compiler_params=pltpu.CompilerParams(vmem_limit_bytes=64 * 1024 * 1024),
    )(q.reshape(n_heads, sq, d), k.reshape(n_heads, sk, d), v.reshape(n_heads, sk, d))
    return out.reshape(b, h, sq, d)
```

```python
import functools

import jax
import jax.numpy as jnp
import jax.experimental.pallas as pl
import jax.experimental.pallas.tpu as pltpu

_LOG2E = 1.4426950408889634

_K = 4
_RING = 4
_RROWS = 32
_RHEADS = 2
_WK = 8
_WROWS = 32
_BACK = 2
_RTHREAD = (1, 0, 1)


def _attention_head(q, k, v, scale):
    s = jax.lax.dot_general(
        q, k, (((1,), (1,)), ((), ())), preferred_element_type=jnp.float32)
    m = jnp.max(s, axis=-1, keepdims=True)
    p = jnp.exp2((s - m) * (scale * _LOG2E))
    l = jnp.sum(p, axis=-1, keepdims=True)
    o = jnp.dot(p.astype(v.dtype), v, preferred_element_type=jnp.float32)
    return o * (1.0 / l)


def _kernel(q_hbm, k_hbm, v_hbm, o_hbm, in_buf, out_buf, in_sem, out_sem, *,
            scale):
    n_chunks, seq = q_hbm.shape[1], q_hbm.shape[2]
    n_cols = out_buf.shape[1]
    srcs = (q_hbm, k_hbm, v_hbm)

    def start_reads(j, slot):
        for r0 in range(0, seq, _RROWS):
            rows = pl.ds(r0, _RROWS)
            for h0 in range(0, _K, _RHEADS):
                heads = pl.ds(h0, _RHEADS)
                for a, src in enumerate(srcs):
                    pltpu.make_async_copy(
                        src.at[heads, j, rows, :],
                        in_buf.at[slot, a, heads, rows, :],
                        in_sem.at[slot],
                    ).start(priority=_RTHREAD[a])

    def wait_reads(slot):
        pltpu.make_async_copy(
            in_buf.at[slot], in_buf.at[slot], in_sem.at[slot]).wait()

    def start_writes(c):
        for r0 in range(0, seq, _WROWS):
            rows = pl.ds(r0, _WROWS)
            pltpu.make_async_copy(
                out_buf.at[:, c, rows, :], o_hbm.at[:, c, rows, :],
                out_sem.at[0]).start()

    write_at = n_chunks - _BACK
    early_cols = n_cols - _BACK

    for j in range(_RING):
        start_reads(j, j)

    def step(j, carry):
        slot = j % _RING
        wait_reads(slot)

        @pl.when(j == write_at)
        def _():
            def write_col(c, cc):
                start_writes(c)
                return cc
            jax.lax.fori_loop(0, early_cols, write_col, 0)

        for h in range(_K):
            o = _attention_head(
                in_buf[slot, 0, h], in_buf[slot, 1, h], in_buf[slot, 2, h], scale)
            head = h * n_chunks + j
            out_buf[head // n_cols, head % n_cols] = o.astype(out_buf.dtype)

        @pl.when(j + _RING < n_chunks)
        def _():
            start_reads(j + _RING, slot)

        return carry

    jax.lax.fori_loop(0, n_chunks, step, 0)

    for c in range(early_cols, n_cols):
        start_writes(c)
    pltpu.make_async_copy(out_buf, o_hbm, out_sem.at[0]).wait()


@jax.jit
def pallas_standalone__mha_softmax__near_ridge_kernel(
    q: jax.Array,
    k: jax.Array,
    v: jax.Array,
):
    b, h, s, d = q.shape
    assert q.shape == k.shape == v.shape and q.dtype == k.dtype == v.dtype
    n_heads = b * h
    n_chunks, n_cols = n_heads // _K, n_heads // _WK
    assert n_chunks * _K == n_heads and n_cols * _WK == n_heads
    assert s % _RROWS == 0 and s % _WROWS == 0 and _K % _RHEADS == 0
    assert n_chunks % n_cols == 0
    assert _BACK <= _RING < n_chunks and 1 <= _BACK < n_cols

    chunk_view = (_K, n_chunks, s, d)
    any_spec = pl.BlockSpec(memory_space=pl.ANY)
    out = pl.pallas_call(
        functools.partial(_kernel, scale=d ** -0.5),
        in_specs=[any_spec, any_spec, any_spec],
        out_specs=any_spec,
        out_shape=jax.ShapeDtypeStruct((_WK, n_cols, s, d), q.dtype),
        scratch_shapes=[
            pltpu.VMEM((_RING, 3, _K, s, d), q.dtype),
            pltpu.VMEM((_WK, n_cols, s, d), q.dtype),
            pltpu.SemaphoreType.DMA((_RING,)),
            pltpu.SemaphoreType.DMA((1,)),
        ],
        compiler_params=pltpu.CompilerParams(
            vmem_limit_bytes=64 * 1024 * 1024,
            disable_bounds_checks=True,
        ),
    )(q.reshape(chunk_view), k.reshape(chunk_view), v.reshape(chunk_view))
    return out.reshape(b, h, s, d)
```

```python
import functools

import jax
import jax.numpy as jnp
import jax.experimental.pallas as pl
import jax.experimental.pallas.tpu as pltpu

_LOG2E = 1.4426950408889634

_K = 4
_RING = 4
_RROWS = 32
_RHEADS = 2
_WK = 8
_WROWS = 32
_BACK = 2
_RTHREAD = (1, 0, 1)


def _attention_head(q, k, v, scale):
    s = jax.lax.dot_general(
        q, k, (((1,), (1,)), ((), ())), preferred_element_type=jnp.float32)
    m = jnp.max(s, axis=-1, keepdims=True)
    p = jnp.exp2((s - m) * (scale * _LOG2E))
    l = jnp.sum(p, axis=-1, keepdims=True)
    o = jnp.dot(p.astype(v.dtype), v, preferred_element_type=jnp.float32)
    return o * (1.0 / l)


def _kernel(q_hbm, k_hbm, v_hbm, o_hbm, in_buf, out_buf, in_sem, out_sem, *,
            scale):
    n_chunks, seq = q_hbm.shape[1], q_hbm.shape[2]
    n_cols = out_buf.shape[1]
    srcs = (q_hbm, k_hbm, v_hbm)

    def start_reads(j, slot):
        for r0 in range(0, seq, _RROWS):
            rows = pl.ds(r0, _RROWS)
            for h0 in range(0, _K, _RHEADS):
                heads = pl.ds(h0, _RHEADS)
                for a, src in enumerate(srcs):
                    pltpu.make_async_copy(
                        src.at[heads, j, rows, :],
                        in_buf.at[slot, a, heads, rows, :],
                        in_sem.at[slot],
                    ).start(priority=_RTHREAD[a])

    def wait_reads(slot):
        pltpu.make_async_copy(
            in_buf.at[slot], in_buf.at[slot], in_sem.at[slot]).wait()

    def start_writes(c):
        for r0 in range(0, seq, _WROWS):
            rows = pl.ds(r0, _WROWS)
            pltpu.make_async_copy(
                out_buf.at[:, c, rows, :], o_hbm.at[:, c, rows, :],
                out_sem.at[0]).start()

    write_at = n_chunks - _BACK
    early_cols = n_cols - _BACK

    for j in range(_RING):
        start_reads(j, j)

    def step(j, carry):
        slot = j % _RING
        wait_reads(slot)

        @pl.when(j == write_at)
        def _():
            def write_col(c, cc):
                start_writes(c)
                return cc
            jax.lax.fori_loop(0, early_cols, write_col, 0)

        for h in range(_K):
            o = _attention_head(
                in_buf[slot, 0, h], in_buf[slot, 1, h], in_buf[slot, 2, h], scale)
            head = h * n_chunks + j
            out_buf[head // n_cols, head % n_cols] = o.astype(out_buf.dtype)

        for free in range(_RING):
            @pl.when(jnp.logical_and(slot == free, j + _RING < n_chunks))
            def _(free=free):
                start_reads(j + _RING, free)

        return carry

    jax.lax.fori_loop(0, n_chunks, step, 0)

    for c in range(early_cols, n_cols):
        start_writes(c)
    pltpu.make_async_copy(out_buf, o_hbm, out_sem.at[0]).wait()


@jax.jit
def pallas_standalone__mha_softmax__near_ridge_kernel(
    q: jax.Array,
    k: jax.Array,
    v: jax.Array,
):
    b, h, s, d = q.shape
    assert q.shape == k.shape == v.shape and q.dtype == k.dtype == v.dtype
    n_heads = b * h
    n_chunks, n_cols = n_heads // _K, n_heads // _WK
    assert n_chunks * _K == n_heads and n_cols * _WK == n_heads
    assert s % _RROWS == 0 and s % _WROWS == 0 and _K % _RHEADS == 0
    assert n_chunks % n_cols == 0
    assert _BACK <= _RING < n_chunks and 1 <= _BACK < n_cols

    chunk_view = (_K, n_chunks, s, d)
    any_spec = pl.BlockSpec(memory_space=pl.ANY)
    out = pl.pallas_call(
        functools.partial(_kernel, scale=d ** -0.5),
        in_specs=[any_spec, any_spec, any_spec],
        out_specs=any_spec,
        out_shape=jax.ShapeDtypeStruct((_WK, n_cols, s, d), q.dtype),
        scratch_shapes=[
            pltpu.VMEM((_RING, 3, _K, s, d), q.dtype),
            pltpu.VMEM((_WK, n_cols, s, d), q.dtype),
            pltpu.SemaphoreType.DMA((_RING,)),
            pltpu.SemaphoreType.DMA((1,)),
        ],
        compiler_params=pltpu.CompilerParams(vmem_limit_bytes=64 * 1024 * 1024),
    )(q.reshape(chunk_view), k.reshape(chunk_view), v.reshape(chunk_view))
    return out.reshape(b, h, s, d)
```
